```python
import os as _os
_os.environ.setdefault("JAX_PLATFORMS", "cpu")
import jax
import jax.numpy as jnp

def _softmax(x, axis=-1):
    return jax.nn.softmax(x, axis=axis)
def _gelu(x):
    return jax.nn.gelu(x, approximate=True)
def _silu(x):
    return jax.nn.silu(x)
def _sigmoid(x):
    return jax.nn.sigmoid(x)
def _layernorm(x, axis=-1, eps=1e-5):
    m = jnp.mean(x, axis=axis, keepdims=True)
    v = jnp.var(x, axis=axis, keepdims=True)
    return (x - m) / jnp.sqrt(v + eps)
def _scatter_add(tgt, idx, src, axis=0):
    return tgt.at[idx].add(src)
def _segment_sum(src, seg, n):
    return jax.ops.segment_sum(src, seg, n)
class _Rng:
    def __init__(self, key):
        self._k = key
    def _next(self):
        self._k, sub = jax.random.split(self._k)
        return sub
    def normal(self, shape):
        return jax.random.normal(self._next(), shape, dtype=jnp.bfloat16)
    def randint(self, lo, hi, shape):
        return jax.random.randint(self._next(), shape, lo, hi, dtype=jnp.int32)
    def uniform(self, shape, lo=0.0, hi=1.0):
        return jax.random.uniform(self._next(), shape, jnp.bfloat16, lo, hi)
    def permutation(self, n):
        return jax.random.permutation(self._next(), n)


kernel_name = 'concat_heads__ssm_conv_s4__grouped_kv_mqa__prompt'

def setup_inputs():
    _rng = _Rng(jax.random.key(int.from_bytes(__import__("os").urandom(4), "little")))
    _w = (lambda a: (lambda t: t.astype(jnp.bfloat16) if jnp.issubdtype(t.dtype, jnp.floating) else t)(jnp.asarray(a)))
    def _A_setup():
        B, L, D, N = 1, 2048, 448, 256
        A_re = -jnp.exp((lambda *s: _rng.normal(s) * 0.1)(D, N))
        A_im = jnp.pi * (lambda *s: _rng.normal(s) * 0.1)(D, N)
        B_re = (lambda *s: _rng.normal(s) * 0.1)(D, N)
        B_im = (lambda *s: _rng.normal(s) * 0.1)(D, N)
        C_re = (lambda *s: _rng.normal(s) * 0.1)(D, N)
        C_im = (lambda *s: _rng.normal(s) * 0.1)(D, N)
        log_dt = (lambda *s: _rng.normal(s) * 0.1)(D) * 0.5 - 4.0
        Dskip = (lambda *s: _rng.normal(s) * 0.05)(D)
        return {
            "u": _w((lambda *s: _rng.normal(s) * 0.05)(B, L, D)),
            "A_re": _w(A_re),
            "A_im": _w(A_im),
            "B_re": _w(B_re),
            "B_im": _w(B_im),
            "C_re": _w(C_re),
            "C_im": _w(C_im),
            "log_dt": _w(log_dt),
            "Dskip": _w(Dskip),
        }
    _A_in = _A_setup()

    def _B_setup():
        B, S, D, H = 1, 2048, 448, 16
        Dh = D // H
        return {
            "x": _w((lambda *s: _rng.normal(s) * 0.05)(B, S, D)),
            "wq": _w((lambda *s: _rng.normal(s) * 0.8)(D, H * Dh)),
            "wk": _w((lambda *s: _rng.normal(s) * 0.8)(D, Dh)),
            "wv": _w((lambda *s: _rng.normal(s) * 0.05)(D, Dh)),
            "wo": _w((lambda *s: _rng.normal(s) * 0.05)(H * Dh, D)),
        }
    _B_in = _B_setup()

    return {
        "A_u": _A_in["u"],
        "A_A_re": _A_in["A_re"],
        "A_A_im": _A_in["A_im"],
        "A_B_re": _A_in["B_re"],
        "A_B_im": _A_in["B_im"],
        "A_C_re": _A_in["C_re"],
        "A_C_im": _A_in["C_im"],
        "A_log_dt": _A_in["log_dt"],
        "A_Dskip": _A_in["Dskip"],
        "B_x": _B_in["x"],
        "B_wq": _B_in["wq"],
        "B_wk": _B_in["wk"],
        "B_wv": _B_in["wv"],
        "B_wo": _B_in["wo"],
    }

def reference(A_u, A_A_re, A_A_im, A_B_re, A_B_im, A_C_re, A_C_im, A_log_dt, A_Dskip, B_x, B_wq, B_wk, B_wv, B_wo):
    def _A_ref(u, A_re, A_im, B_re, B_im, C_re, C_im, log_dt, Dskip):
        Bsz, L, D = u.shape
        dt = jnp.exp(log_dt)[:, None]
        A = A_re + 1j * A_im
        Bc = B_re + 1j * B_im
        Cc = C_re + 1j * C_im
        logdA = dt * A
        dB = dt * Bc
        l = (lambda x, dt: x.astype(dt))(jnp.arange(L), A_re.dtype)
        P = jnp.exp(logdA[:, :, None] * l[None, None, :])
        K = jnp.einsum("dn,dnl,dn->dl", Cc, P, dB).real
        L2 = 2 * L
        Kp = jnp.pad(K, ((0, 0), (0, L)))
        up = (lambda x, *d: x.transpose(*d))(u, 0, 2, 1)
        up = jnp.pad(up, ((0, 0), (0, 0), (0, L)))
        Kf = (lambda x, axes=(-2,-1): jnp.fft.rfft2(x.astype(jnp.float32), axes=axes))(Kp[:, None, :], axes=(-2, -1))
        Uf = (lambda x, axes=(-2,-1): jnp.fft.rfft2(x.astype(jnp.float32), axes=axes))(up[:, :, None, :], axes=(-2, -1))
        Yf = Uf * Kf[None, :, :, :]
        y = (lambda x, s, axes=(-2,-1): jnp.fft.irfft2(x, s=s, axes=axes).astype(jnp.bfloat16))(Yf, (1, L2), axes=(-2, -1))[:, :, 0, :L]
        y = (lambda x, *d: x.transpose(*d))(y, 0, 2, 1) + u * Dskip[None, None, :]
        return y

    def _B_ref(x, wq, wk, wv, wo):
        B, S, D = x.shape
        H = 16
        Dh = D // H
        q = (lambda x, *d: x.transpose(*d))((x @ wq).reshape(B, S, H, Dh), 0, 2, 1, 3)
        k = x @ wk
        v = x @ wv
        scores = jnp.einsum("bhqd,bkd->bhqk", q, k) * (Dh ** -0.5)
        p = _softmax(scores, axis=-1)
        o = jnp.einsum("bhqk,bkd->bhqd", p, v)
        return (lambda x, *d: x.transpose(*d))(o, 0, 2, 1, 3).reshape(B, S, H * Dh) @ wo

    a = _A_ref(A_u, A_A_re, A_A_im, A_B_re, A_B_im, A_C_re, A_C_im, A_log_dt, A_Dskip)
    b = _B_ref(B_x, B_wq, B_wk, B_wv, B_wo)
    return jnp.concatenate([a, b], axis=-1)
```

```python
import functools

import ml_dtypes
import numpy as np

import jax
import jax.numpy as jnp
import jax.experimental.pallas as pl
import jax.experimental.pallas.tpu as pltpu

L = 2048
D = 448
N = 256
H = 16
DH = D // H
T = 128
NC = L // T
NU = 64
AP = 48
AS, BS, KS = 49, 17, 529
KPAD = 16
PACE_BASES = (16, 2, 0)
PACE_KGEN = (14, 4, 1)
PACE_MIX = (16, 16, 0)
X_BLOCKS = ((0, 256), (256, 768), (1024, 1024))
KG_CH = 16
KF0 = 8
ITEM_ROWS = NC * 2 * 8
ITEMS = 56
UF0 = KF0 + ITEMS * ITEM_ROWS + 16
STAGE0 = UF0 + ITEMS * ITEM_ROWS
POS_ROWS = 26 * 8
BIG_ROWS = STAGE0 + (D // 8) * 2 * POS_ROWS
F32 = jnp.float32
BF16 = jnp.bfloat16

A_EXPS = (list(range(16)) + [256 + 2 * i for i in range(8)]
          + [512 + 4 * i for i in range(4)] + [768 + 4 * i for i in range(4)]
          + [1024 + 256 * j + 8 * i for j in range(4) for i in range(2)] + [2048])


def _chunk_pieces(c):
    if c < 2:
        return [(8 * c + b, r) for b in range(8) for r in (0, 8)]
    group = lambda cc: 16 if cc < 4 else 24 if cc < 8 else 32 if cc < 16 else 40
    b0 = 8 * (c % 2)
    extra = (8, group(c)) if c % 2 == 0 else (0, group(c + 1))
    return [(b0 + b, group(c)) for b in range(8)] + [extra, extra]


def _constants():
    even = np.arange(0, T, 2)
    freq = np.concatenate([even, T - 1 - even])
    omega = 2.0 * np.pi * (freq + 0.5) / (2 * T)
    ang = omega[:, None] * np.arange(T)[None, :]
    fwd = np.concatenate([np.cos(ang), -np.sin(ang)], axis=0)
    pos = np.arange(L).astype(np.float32).astype(ml_dtypes.bfloat16).astype(np.int64)
    fk = np.zeros((NC, 2 * T, T), np.float64)
    for c in range(NC):
        where = {}
        for p, (b, r) in enumerate(_chunk_pieces(c)):
            for i in range(8):
                if r + i < len(A_EXPS):
                    where.setdefault(A_EXPS[r + i] + 16 * b, 8 * p + i)
        for j in range(T):
            fk[c, :, where[int(pos[c * T + j])]] += fwd[:, j]
    inv = []
    for parity in range(2):
        a = omega[None, :T // 2] * np.arange(parity, T, 2)[:, None]
        inv.append(np.concatenate([np.cos(a), -np.sin(a)], axis=1) / T)

    def packed(v):
        bits = v.astype(np.float32).astype(ml_dtypes.bfloat16).view(np.uint16).astype(np.uint32)
        return bits[..., 0::2, :] | (bits[..., 1::2, :] << 16)
    return packed(fwd), packed(fk), packed(np.concatenate(inv, axis=0))


_FWD, _FK, _INV = _constants()


def _cmul(x, y):
    return x[0] * y[0] - x[1] * y[1], x[0] * y[1] + x[1] * y[0]


def _csq(x):
    t = x[0] * x[1]
    return (x[0] + x[1]) * (x[0] - x[1]), t + t


def _round8(n):
    return -(-n // 8) * 8


def _aligned(start, size):
    return pl.ds(start if isinstance(start, int) else pl.multiple_of(start, size), size)


def _dot(a, b):
    return jnp.dot(a, b, preferred_element_type=F32)


def _dot_nt(a, b):
    return jax.lax.dot_general(a, b, (((1,), (1,)), ((), ())), preferred_element_type=F32)


def _kernel(u_hbm, are_hbm, aim_hbm, bre_hbm, bim_hbm, cre_hbm, cim_hbm, ldt_hbm, dsk_hbm,
            x_hbm, wq_hbm, wk_hbm, wv_hbm, wo_hbm, fwd_hbm, fk_hbm, inv_hbm,
            out_hbm,
            u_v, par_v, ldt_v, dsk_v, x_v, wq_v, wk_v, wv_v, wo_v, fwd_v, fk_v, inv_v,
            wt_v, wos_v, wot_v, dt_v, q_v, k_v, vt_v, s_v, acc_v, qt_v, big_v, ot_v,
            a_v, b_v, kraw_v, kt_v, yf_v, o_v, in_sem, out_sem):
    XB = len(X_BLOCKS)
    copies = [(wq_hbm, wq_v), (wk_hbm, wk_v), (wv_hbm, wv_v)]
    copies += [(x_hbm.at[0, :, pl.ds(x0, n)], x_v.at[:, pl.ds(x0, n)]) for x0, n in X_BLOCKS]
    copies += [(r, par_v.at[i]) for i, r in
               enumerate((are_hbm, aim_hbm, bre_hbm, bim_hbm, cre_hbm, cim_hbm))]
    copies += [(ldt_hbm, ldt_v), (dsk_hbm, dsk_v)]
    copies += [(u_hbm.at[0], u_v), (fwd_hbm, fwd_v), (fk_hbm, fk_v), (inv_hbm, inv_v), (wo_hbm, wo_v)]
    dmas = [pltpu.make_async_copy(s, d, in_sem.at[i]) for i, (s, d) in enumerate(copies)]
    for d in dmas:
        d.start()
    w_dma, x_dma, par_dma = dmas[:3], dmas[3:3 + XB], dmas[3 + XB:11 + XB]
    late_dma = dmas[11 + XB:]

    for d in w_dma:
        d.wait()
    wq = wq_v[...].astype(F32)
    wq = jnp.concatenate([wq, jnp.zeros((D, 4 * T - D), F32)], axis=1)
    wt_v[0:D // 2, :] = pltpu.bitcast(wq.T[0:D].astype(BF16), jnp.uint32)
    for i, w_ref in enumerate((wk_v, wv_v)):
        w = jnp.concatenate([w_ref[...].astype(F32), jnp.zeros((32 - DH, D), F32)], axis=0)
        wt_v[D // 2 + 16 * i:D // 2 + 16 * (i + 1), :] = pltpu.bitcast(w.astype(BF16), jnp.uint32)

    def bases(g, half, lt):
        def run():
            par = [par_v[i, _aligned(16 * g, 16), lt * T:(lt + 1) * T].astype(F32)[8 * half:8 * half + 8]
                   for i in range(6)]
            dtc = dt_v[_aligned(8 + 16 * g + 8 * half, 8), :]
            mag = jnp.exp(dtc * par[0])
            ph = dtc * par[1]
            val = {0: _cmul((par[4], par[5]), (dtc * par[2], dtc * par[3])),
                   1: (mag * jnp.cos(ph), mag * jnp.sin(ph))}
            e = 1
            while e < L:
                val[2 * e] = _csq(val[e])
                e *= 2
            for e, v in val.items():
                for ri in range(2):
                    row = STAGE0 + (4 * g + 2 * half + lt) * POS_ROWS + 16 * e.bit_length() + 8 * ri
                    big_v[_aligned(row, 8), :] = v[ri]
        return run

    q_scale = float(DH ** -0.5 * np.log2(np.e))
    for i, (x0, n) in enumerate(X_BLOCKS):
        x_dma[i].wait()
        for c0 in range(x0, x0 + n, 4 * T):
            w = min(4 * T, x0 + n - c0)
            r = _dot(pltpu.bitcast(wt_v[...], BF16), x_v[:, c0:c0 + w])
            for j in range(w // T):
                q_v[c0 // T + j] = r[:, j * T:(j + 1) * T] * q_scale
            kt = jnp.concatenate([r[D:D + 32], jnp.zeros((T - 32, w), F32)], axis=0)
            k_v[c0 // 2:(c0 + w) // 2, :] = pltpu.bitcast(kt.T[:, 0:32].astype(BF16), jnp.uint32)
            ones_row = jax.lax.broadcasted_iota(jnp.int32, (32, w), 0) == DH
            vt_v[:, c0:c0 + w] = pltpu.bitcast(
                jnp.where(ones_row, 1.0, r[D + 32:D + 64]).astype(BF16), jnp.uint32)

    a_v[...] = jnp.zeros(a_v.shape, F32)
    b_v[0:2] = jnp.ones((2,) + b_v.shape[1:], F32)
    b_v[2:4] = jnp.zeros((2,) + b_v.shape[1:], F32)
    for b in range(16):
        kraw_v[pl.ds(b * KS + KPAD + D, 4 * T - D), :] = jnp.zeros((4 * T - D, T), F32)
    for d in par_dma:
        d.wait()
    dt = jnp.exp(ldt_v[...].astype(F32).reshape(1, D)).astype(BF16).astype(F32)
    dskip = jnp.concatenate(
        [dsk_v[...].astype(F32).reshape(1, D), jnp.zeros((1, 4 * T - D), F32)], axis=1)
    dt = jnp.concatenate([dt, jnp.zeros((1, 4 * T - D), F32)], axis=1)
    dt_v[8:, :] = jnp.broadcast_to(dt, (T, 4 * T)).T

    def load_queries(u):
        t, g = u // 4, u % 4
        return jnp.concatenate(
            [q_v[t, pl.ds(4 * DH * g + DH * i, 32), :] for i in range(4)], axis=1).astype(BF16)

    def normalise(u):
        acc = acc_v[...]
        o = (acc * (1.0 / acc[DH:DH + 1, :])).astype(BF16)
        for i in range(4):
            ot_v[u + 1, 32 * i:32 * (i + 1), :] = o[:, i * T:(i + 1) * T]

    def attention(u, m_prev, scores=True, values=True, side_work=(), pace=None, mark_ref=big_v):
        if scores:
            qt = pltpu.bitcast(qt_v[...], BF16)
        if values:
            m_prev = jnp.max(m_prev, axis=0, keepdims=True)
        m_run = None
        for j in range(NC):
            rows = slice(j * T, (j + 1) * T)
            if scores:
                kc = pltpu.bitcast(k_v[j * T // 2:(j + 1) * T // 2, :], BF16)
                s = _dot(kc, qt)
            if values:
                p = jnp.exp2(s_v[rows, :] - m_prev).astype(BF16)
                d = _dot(pltpu.bitcast(vt_v[:, rows], BF16), p)
                if j == 0:
                    normalise(u - 2)
                acc_v[...] = d if j == 0 else acc_v[...] + d
            if scores:
                s_v[rows, :] = s
                cm = jnp.max(s.reshape(T // 8, 8, 4 * T), axis=0)
                m_run = cm if m_run is None else jnp.maximum(m_run, cm)
                if j == 12:
                    q_next = load_queries(jnp.minimum(u + 1, NU - 1))
            if side_work and j < pace[0]:
                n = pace[0] * pace[1]
                for i in range(pace[1]):
                    k = j * pace[1] + i
                    for w in side_work[k * len(side_work) // n:(k + 1) * len(side_work) // n]:
                        w()
                    r = i * T // pace[1] // 8 * 8
                    mark_ref[0:8, :] = s[r:r + 8, pace[2] * T:(pace[2] + 1) * T]
        if scores:
            qt_v[...] = pltpu.bitcast(q_next, jnp.uint32)
            return m_run

    def contract(c0, pair):
        def run():
            def gather(ref, pitch, n):
                return jnp.concatenate(
                    [jnp.concatenate([ref[i, pl.ds(pitch * ch, n), :] for i in range(4)], axis=1)
                     for ch in (2 * pair, 2 * pair + 1)], axis=0).astype(BF16)
            am = gather(a_v, AS, AP)
            bm = gather(b_v, BS, 16)
            r = _dot_nt(bm, am)
            r = jnp.concatenate([r, jnp.zeros((32, T - 2 * AP), F32)], axis=1)
            for ch in range(2):
                for hb in range(2):
                    kraw_v[pl.ds(8 * hb * KS + KPAD + c0 + 2 * pair + ch, 8, stride=KS), :] = (
                        r[16 * ch + 8 * hb:16 * ch + 8 * hb + 8])
        return run

    def kgen_work(step):
        c0 = pl.multiple_of(step * KG_CH, KG_CH)

        def powers(half, lt):
            base = STAGE0 + (4 * step + 2 * half + lt) * POS_ROWS

            def get(e):
                row = base + 16 * e.bit_length()
                return tuple(big_v[pl.ds(pl.multiple_of(row + 8 * ri, 8), 8), :] for ri in range(2))

            def put_a(row, val):
                for ri in range(2):
                    a_v[2 * ri + lt, pl.ds(8 * half * AS + row, 8, stride=AS), :] = val[ri]

            pa, pb = {}, {}

            def a_row(row):
                def run():
                    e = A_EXPS[row]
                    low = e & -e
                    if e == 0:
                        pa[e] = get(0)
                    else:
                        pa[e] = _cmul(get(0) if e == low else pa[e - low], get(low))
                    put_a(row, pa[e])
                return run

            def b_row(b):
                def run():
                    low = b & -b
                    zr, zi = get(16 * low)
                    if b == low:
                        pb[b] = (zr, -zi)
                    else:
                        xr_, xi_ = pb[b - low]
                        pb[b] = (xr_ * zr + xi_ * zi, xi_ * zr - xr_ * zi)
                    for ri in range(2):
                        b_v[2 * ri + lt, pl.ds(8 * half * BS + b, 8, stride=BS), :] = pb[b][ri]
                return run

            return [b_row(b) for b in range(1, 16)] + [a_row(r) for r in range(len(A_EXPS))]

        both = lambda f, g: (lambda: (f(), g()))
        work = powers(0, 0) + powers(0, 1) + powers(1, 0) + powers(1, 1)
        n = len(work) // 8
        for p in range(4):
            work[n * p] = both(contract(c0 - KG_CH, 4 + p), work[n * p])
            work[n * (4 + p)] = both(contract(c0, p), work[n * (4 + p)])
        return work

    def spectra():
        odd_lane = jax.lax.broadcasted_iota(jnp.int32, (AP, T), 1) % 2 == 1
        for b in range(16):
            for ct in range(4):
                r = kraw_v[pl.ds(b * KS + KPAD + ct * T, T), :].T
                kt_v[b, :, ct * T:(ct + 1) * T] = jnp.where(odd_lane, r[AP:2 * AP], r[0:AP])
        h = T // 2
        low = jax.lax.broadcasted_iota(jnp.int32, (h, T), 1) < h

        def put(base, c, ct, ri, val):
            for rv in range(val.shape[0] // 8):
                row = base + (16 * ct + rv) * ITEM_ROWS + 16 * c + 8 * ri
                big_v[row:row + 8, :] = val[8 * rv:8 * rv + 8]

        tiles = [(c, ct) for c in range(NC) for ct in range(4) if ct < 3 or c % 2 == 0]
        fwd = pltpu.bitcast(fwd_v[...], BF16)
        for i in range(0, len(tiles), 4):
            rhs = [u_v[ct * T:(ct + 1) * T, c * T:(c + 1) * T] if ct < 3 else
                   jnp.concatenate([u_v[3 * T:D, cc * T:(cc + 1) * T] for cc in (c, c + 1)], axis=0)
                   for c, ct in tiles[i:i + 4]]
            uf = _dot_nt(fwd, jnp.concatenate(rhs, axis=0))
            for k, (c, ct) in enumerate(tiles[i:i + 4]):
                r = uf[:, k * T:(k + 1) * T]
                if ct < 3:
                    put(UF0, c, ct, 0, r[0:T])
                    put(UF0, c, ct, 1, r[T:])
                    continue
                for ri in range(2):
                    ra, rb = r[ri * T:ri * T + h], r[ri * T + h:(ri + 1) * T]
                    put(UF0, c, 3, ri, jnp.where(low, ra, pltpu.roll(rb, h, 1)))
                    put(UF0, c + 1, 3, ri, jnp.where(low, pltpu.roll(ra, h, 1), rb))
        prev = None
        for c in range(NC):
            pieces = _chunk_pieces(c)
            kd = jnp.concatenate([kt_v[b, r:r + 8, :] for b, r in pieces], axis=0).astype(BF16)
            kf = _dot(pltpu.bitcast(fk_v[c, :, 0:8 * len(pieces)], BF16), kd)
            if c == 0:
                kf = jnp.concatenate([kf[0:T] + dskip, kf[T:]], axis=0)
            seg = kf
            if prev is not None:
                seg = jnp.concatenate(
                    [kf[0:h] - prev[2 * h:3 * h], kf[h:2 * h] + prev[3 * h:],
                     kf[2 * h:3 * h] + prev[0:h], kf[3 * h:] - prev[h:2 * h]], axis=0)
            for ct in range(3):
                put(KF0, c, ct, 0, seg[0:T, ct * T:(ct + 1) * T])
                put(KF0, c, ct, 1, seg[T:, ct * T:(ct + 1) * T])
            for ri in range(2):
                ra, rb = seg[ri * T:ri * T + h, 3 * T:], seg[ri * T + h:(ri + 1) * T, 3 * T:]
                put(KF0, c, 3, ri, jnp.where(low, ra, pltpu.roll(rb, h, 1)))
            prev = kf

    def mix_work(step):
        def outputs(item, a):
            def load(base, c):
                row = base + item * ITEM_ROWS + 16 * c
                return big_v[_aligned(row, 8), :], big_v[_aligned(row + 8, 8), :]

            acc = {a: None, a + 1: None}
            state = {"u": None}

            def term(c):
                def run():
                    u_hi = state["u"]
                    kr, ki = load(KF0, c)
                    ks, kd = kr + ki, ki - kr
                    if u_hi is None:
                        ur, ui = load(UF0, a + 1)
                        u_hi = (ur, ui, ur + ui)
                    u_lo = None
                    if c <= a:
                        ur, ui = load(UF0, a - c)
                        u_lo = (ur, ui, ur + ui)
                    for o, uu in ((a + 1, u_hi), (a, u_lo)):
                        if uu is not None:
                            p = (kr * uu[2], uu[1] * ks, uu[0] * kd)
                            acc[o] = p if acc[o] is None else tuple(x + y for x, y in zip(acc[o], p))
                    state["u"] = u_lo
                    if c == a + 1:
                        for o, (t1, t2, t3) in acc.items():
                            yf_v[item, 16 * o:16 * o + 8, :] = t1 - t2
                            yf_v[item, 16 * o + 8:16 * o + 16, :] = t1 + t3
                return run
            return [term(c) for c in range(a + 2)]

        work = []
        for p in range(NC // 2):
            work += outputs(2 * step, NC - 2 - 2 * p) + outputs(2 * step + 1, 2 * p)
        return work

    def ssm_output(c0, nc):
        h = T // 2
        low = jax.lax.broadcasted_iota(jnp.int32, (h, T), 1) < h
        tiles = [(c, ct) for c in range(c0, c0 + nc) for ct in range(4) if ct < 3 or c % 2 == 0]
        parts = [[], []]
        get = lambda c, item, ri: jnp.concatenate(
            [yf_v[item + rv, 16 * c + 8 * ri:16 * c + 8 * ri + 8, :] for rv in range(8)], axis=0)
        for c, ct in tiles:
            quarter = []
            for ri in range(2):
                if ct < 3:
                    quarter += [get(c, 16 * ct, ri), get(c, 16 * ct + 8, ri)]
                else:
                    x0, x1 = get(c, 48, ri), get(c + 1, 48, ri)
                    quarter += [jnp.where(low, x0, pltpu.roll(x1, h, 1)),
                                jnp.where(low, pltpu.roll(x0, h, 1), x1)]
            parts[0].append(jnp.concatenate([quarter[0] + quarter[1], quarter[2] - quarter[3]], axis=0))
            parts[1].append(jnp.concatenate([quarter[0] - quarter[1], quarter[2] + quarter[3]], axis=0))
        y = [_dot(pltpu.bitcast(inv_v[parity * h // 2:(parity + 1) * h // 2, :], BF16),
                  jnp.concatenate(parts[parity], axis=1).astype(BF16)) for parity in range(2)]
        for k, (c, ct) in enumerate(tiles):
            even, odd = (pltpu.bitcast(
                y[parity][:, k * T:(k + 1) * T].astype(BF16).astype(F32), jnp.uint32) for parity in range(2))
            words = odd | (even >> 16)
            if ct < 3:
                o_v[c * T:(c + 1) * T, ct * T:(ct + 1) * T] = pltpu.bitcast(words, BF16)
            else:
                o_v[c * T:(c + 1) * T, 3 * T:D] = pltpu.bitcast(words, BF16)[:, 0:h]
                o_v[(c + 1) * T:(c + 2) * T, 3 * T:D] = pltpu.bitcast(pltpu.roll(words, h, 1), BF16)[:, 0:h]

    def prepare_wo():
        wos_v[0:D, :] = jnp.concatenate([wo_v[...].astype(F32), jnp.zeros((D, 4 * T - D), F32)], axis=1)
        wos_v[D:, :] = jnp.zeros((8, 4 * T), F32)
        keep = jax.lax.broadcasted_iota(jnp.int32, (32, 4 * T), 0) < DH
        w = jnp.concatenate([jnp.where(keep, wos_v[DH * h:DH * h + 32, :], 0.0) for h in range(H)], axis=0)
        wot_v[...] = pltpu.bitcast(w.T[0:D].astype(BF16), jnp.uint32)

    def project(t0, half):
        o = jnp.concatenate(
            [jnp.concatenate([ot_v[4 * t + g + 1] for g in range(4)], axis=0) for t in range(t0, t0 + 4)],
            axis=1)
        pad = 4 * T - D
        cut = (2 * T - pad) // 2
        r = _dot(pltpu.bitcast(wot_v[cut:, :] if half else wot_v[0:cut, :], BF16), o)
        rows = slice(t0 * T, (t0 + 4) * T)
        if half:
            o_v[rows, 5 * T:] = r.T.astype(BF16)
        else:
            r = jnp.concatenate([jnp.zeros((pad, 4 * T), F32), r], axis=0).T.astype(BF16)
            o_v[rows, D:4 * T] = r[:, pad:T]
            o_v[rows, 4 * T:5 * T] = r[:, T:]

    def out_copy(i, t0, nt, c0, nc):
        rows, cols = pl.ds(t0 * T, nt * T), pl.ds(c0 * T, nc * T)
        return pltpu.make_async_copy(o_v.at[rows, cols], out_hbm.at[0, rows, cols], out_sem.at[i])

    def run(lo, hi, m, work, pace, mark_ref=big_v):
        def body(step, m):
            return attention(lo + step, m, side_work=work(step), pace=pace, mark_ref=mark_ref)
        return jax.lax.fori_loop(0, hi - lo, body, m)

    def bases_work(step):
        work = []
        for k in range(16):
            work += [bases(4 * step + k // 4, (k // 2) % 2, k % 2)] + [lambda: None] * 6
        return work

    acc_v[...] = jnp.ones(acc_v.shape, F32)
    qt_v[...] = pltpu.bitcast(load_queries(0), jnp.uint32)
    m = attention(0, None, values=False)
    m = run(1, 8, m, bases_work, PACE_BASES, dt_v)
    for d in late_dma:
        d.wait()
    m = run(8, 36, m, kgen_work, PACE_KGEN)
    for p in range(4):
        contract(D - KG_CH, 4 + p)()
    prepare_wo()
    spectra()
    m = run(36, 50, m, lambda step: mix_work(2 * step) + mix_work(2 * step + 1), PACE_MIX)
    jobs = [functools.partial(ssm_output, c0, 4) for c0 in range(0, NC, 4)]
    jobs += [functools.partial(project, t0, half) for t0 in (0, 4, 8) for half in range(2)]
    stores = ((0, 12, 0, 7), (12, 4, 0, 3), (12, 4, 3, 2), (12, 4, 5, 2))
    for i, job in enumerate(jobs):
        m = attention(50 + i, m)
        job()
    out_copy(0, *stores[0]).start()
    out_copy(1, *stores[1]).start()
    m = jax.lax.fori_loop(50 + len(jobs), NU, attention, m)
    attention(NU, m, scores=False)
    normalise(NU - 1)
    for half in range(2):
        project(12, half)
        out_copy(2 + half, *stores[2 + half]).start()
    for i, block in enumerate(stores):
        out_copy(i, *block).wait()


@jax.jit
def pallas_concat_heads__ssm_conv_s4__grouped_kv_mqa__prompt_kernel(
    A_u: jax.Array,
    A_A_re: jax.Array,
    A_A_im: jax.Array,
    A_B_re: jax.Array,
    A_B_im: jax.Array,
    A_C_re: jax.Array,
    A_C_im: jax.Array,
    A_log_dt: jax.Array,
    A_Dskip: jax.Array,
    B_x: jax.Array,
    B_wq: jax.Array,
    B_wk: jax.Array,
    B_wv: jax.Array,
    B_wo: jax.Array,
):
    hbm = pl.BlockSpec(memory_space=pltpu.HBM)
    scratch = [
        pltpu.VMEM((D, L), BF16),
        pltpu.VMEM((6, D, N), BF16),
        pltpu.VMEM((D,), BF16),
        pltpu.VMEM((D,), BF16),
        pltpu.VMEM((D, L), BF16),
        pltpu.VMEM((D, D), BF16),
        pltpu.VMEM((DH, D), BF16),
        pltpu.VMEM((DH, D), BF16),
        pltpu.VMEM((D, D), BF16),
        pltpu.VMEM((T, T), jnp.uint32),
        pltpu.VMEM((NC, T, T), jnp.uint32),
        pltpu.VMEM((T // 2, T), jnp.uint32),
        pltpu.VMEM((2 * T, D), jnp.uint32),
        pltpu.VMEM((D + 8, 4 * T), F32),
        pltpu.VMEM((D // 2, 4 * T), jnp.uint32),
        pltpu.VMEM((8 + 4 * T, T), F32),
        pltpu.VMEM((NC, 4 * T, T), F32),
        pltpu.VMEM((L // 2, 32), jnp.uint32),
        pltpu.VMEM((16, L), jnp.uint32),
        pltpu.VMEM((L, 4 * T), F32),
        pltpu.VMEM((32, 4 * T), F32),
        pltpu.VMEM((16, 4 * T), jnp.uint32),
        pltpu.VMEM((BIG_ROWS, T), F32),
        pltpu.VMEM((NU + 1, T, T), BF16),
        pltpu.VMEM((4, _round8((KG_CH + 1) * AS), T), F32),
        pltpu.VMEM((4, _round8((KG_CH + 1) * BS), T), F32),
        pltpu.VMEM((_round8(17 * KS), T), F32),
        pltpu.VMEM((16, AP, 4 * T), F32),
        pltpu.VMEM((ITEMS, ITEM_ROWS, T), F32),
        pltpu.VMEM((L, 2 * D), BF16),
        pltpu.SemaphoreType.DMA((16 + len(X_BLOCKS),)),
        pltpu.SemaphoreType.DMA((4,)),
    ]
    return pl.pallas_call(
        _kernel,
        out_shape=jax.ShapeDtypeStruct((1, L, 2 * D), BF16),
        in_specs=[hbm] * 17,
        out_specs=hbm,
        scratch_shapes=scratch,
        compiler_params=pltpu.CompilerParams(
            vmem_limit_bytes=100 * 2 ** 20,
            flags={"XLA_TPU_EVENLY_DISTRIBUTE_CRITICAL_NODES": True}),
    )(A_u.transpose(0, 2, 1), A_A_re, A_A_im, A_B_re, A_B_im, A_C_re, A_C_im,
      A_log_dt, A_Dskip,
      B_x.transpose(0, 2, 1), B_wq, B_wk.T, B_wv.T, B_wo, _FWD, _FK, _INV)
```
